```python
import os as _os
_os.environ.setdefault("JAX_PLATFORMS", "cpu")
import jax
import jax.numpy as jnp

def _softmax(x, axis=-1):
    return jax.nn.softmax(x, axis=axis)
def _gelu(x):
    return jax.nn.gelu(x, approximate=True)
def _silu(x):
    return jax.nn.silu(x)
def _sigmoid(x):
    return jax.nn.sigmoid(x)
def _layernorm(x, axis=-1, eps=1e-5):
    m = jnp.mean(x, axis=axis, keepdims=True)
    v = jnp.var(x, axis=axis, keepdims=True)
    return (x - m) / jnp.sqrt(v + eps)
def _scatter_add(tgt, idx, src, axis=0):
    return tgt.at[idx].add(src)
def _segment_sum(src, seg, n):
    return jax.ops.segment_sum(src, seg, n)
class _Rng:
    def __init__(self, key):
        self._k = key
    def _next(self):
        self._k, sub = jax.random.split(self._k)
        return sub
    def normal(self, shape):
        return jax.random.normal(self._next(), shape, dtype=jnp.bfloat16)
    def randint(self, lo, hi, shape):
        return jax.random.randint(self._next(), shape, lo, hi, dtype=jnp.int32)
    def uniform(self, shape, lo=0.0, hi=1.0):
        return jax.random.uniform(self._next(), shape, jnp.bfloat16, lo, hi)
    def permutation(self, n):
        return jax.random.permutation(self._next(), n)


kernel_name = 'standalone__mha_softmax__near_ridge'

def setup_inputs():
    _rng = _Rng(jax.random.key(int.from_bytes(__import__("os").urandom(4), "little")))
    _w = (lambda a: (lambda t: t.astype(jnp.bfloat16) if jnp.issubdtype(t.dtype, jnp.floating) else t)(jnp.asarray(a)))
    B, H, Sq, Sk, D = 16, 16, 256, 256, 256
    return {
        "q": _w((lambda *s: _rng.normal(s) * 0.4)(B, H, Sq, D)),
        "k": _w((lambda *s: _rng.normal(s) * 0.4)(B, H, Sk, D)),
        "v": _w((lambda *s: _rng.normal(s) * 0.05)(B, H, Sk, D)),
    }

def reference(q, k, v):
    scale = q.shape[-1] ** -0.5
    scores = jnp.einsum("bhqd,bhkd->bhqk", q, k) * scale
    p = _softmax(scores, axis=-1)
    return jnp.einsum("bhqk,bhkd->bhqd", p, v)
```

```python
import functools

import jax
import jax.numpy as jnp
from jax import lax
from jax.experimental import pallas as pl
from jax.experimental.pallas import tpu as pltpu

_HEADS_PER_STEP = 8


def _attn_kernel(q_ref, k_ref, v_ref, o_hbm, acc_ref, sems, *, hb, last, scale):
    i = pl.program_id(0)
    head_cp = pltpu.make_async_copy(
        acc_ref.at[pl.ds(0, last * hb)], o_hbm.at[pl.ds(0, last * hb)], sems.at[0])
    tail_cp = pltpu.make_async_copy(
        acc_ref.at[pl.ds(last * hb, hb)], o_hbm.at[pl.ds(last * hb, hb)], sems.at[1])

    @pl.when(i == last)
    def _():
        head_cp.start()

    for h in range(hb):
        q = q_ref[h]
        k = k_ref[h]
        v = v_ref[h]
        s = lax.dot_general(q, k, (((1,), (1,)), ((), ())),
                            preferred_element_type=jnp.float32) * scale
        m = jnp.max(s, axis=-1, keepdims=True)
        p = jnp.exp(s - m)
        l = jnp.sum(p, axis=-1, keepdims=True)
        o = jnp.dot(p.astype(v.dtype), v, preferred_element_type=jnp.float32)
        acc_ref[i * hb + h] = (o / l).astype(acc_ref.dtype)

    @pl.when(i == last)
    def _():
        tail_cp.start()
        head_cp.wait()
        tail_cp.wait()


@jax.jit
def pallas_standalone__mha_softmax__near_ridge_kernel(
    q: jax.Array,
    k: jax.Array,
    v: jax.Array,
):
    B, H, Sq, D = q.shape
    Sk = k.shape[2]
    BH = B * H
    hb = _HEADS_PER_STEP
    assert BH % hb == 0
    steps = BH // hb
    q2 = q.reshape(BH, Sq, D)
    k2 = k.reshape(BH, Sk, D)
    v2 = v.reshape(BH, Sk, D)
    spec_q = pl.BlockSpec((hb, Sq, D), lambda i: (i, 0, 0))
    spec_kv = pl.BlockSpec((hb, Sk, D), lambda i: (i, 0, 0))
    out = pl.pallas_call(
        functools.partial(_attn_kernel, hb=hb, last=steps - 1, scale=D ** -0.5),
        grid=(steps,),
        in_specs=[spec_q, spec_kv, spec_kv],
        out_specs=pl.BlockSpec(memory_space=pl.ANY),
        out_shape=jax.ShapeDtypeStruct((BH, Sq, D), q.dtype),
        scratch_shapes=[
            pltpu.VMEM((BH, Sq, D), q.dtype),
            pltpu.SemaphoreType.DMA((2,)),
        ],
        compiler_params=pltpu.CompilerParams(
            dimension_semantics=("arbitrary",),
            vmem_limit_bytes=64 * 1024 * 1024,
        ),
    )(q2, k2, v2)
    return out.reshape(B, H, Sq, D)
```

```python
import functools

import jax
import jax.numpy as jnp
from jax import lax
from jax.experimental import pallas as pl
from jax.experimental.pallas import tpu as pltpu

_HEADS_PER_STEP = 8


def _attention_kernel(q_ref, k_ref, v_ref, o_hbm, stage_ref, sems, *, hb, last, scale):
    step = pl.program_id(0)

    tail_copy = pltpu.make_async_copy(
        stage_ref.at[pl.ds(last * hb, hb)],
        o_hbm.at[pl.ds(last * hb, hb)],
        sems.at[1],
    )
    if last > 0:
        head_copy = pltpu.make_async_copy(
            stage_ref.at[pl.ds(0, last * hb)],
            o_hbm.at[pl.ds(0, last * hb)],
            sems.at[0],
        )

    for h in range(hb):
        q = q_ref[h]
        k = k_ref[h]
        v = v_ref[h]
        s = lax.dot_general(
            q, k, (((1,), (1,)), ((), ())), preferred_element_type=jnp.float32
        ) * scale
        m = jnp.max(s, axis=-1, keepdims=True)
        p = jnp.exp(s - m)
        l = jnp.sum(p, axis=-1, keepdims=True)
        o = jnp.dot(p.astype(v.dtype), v, preferred_element_type=jnp.float32)
        stage_ref[step * hb + h] = (o / l).astype(stage_ref.dtype)

    if last > 0:
        @pl.when(step == last - 1)
        def _():
            head_copy.start()

    @pl.when(step == last)
    def _():
        tail_copy.start()
        if last > 0:
            head_copy.wait()
        tail_copy.wait()


def _heads_per_step(bh):
    hb = min(_HEADS_PER_STEP, bh)
    while bh % hb:
        hb -= 1
    return hb


@jax.jit
def pallas_standalone__mha_softmax__near_ridge_kernel(
    q: jax.Array,
    k: jax.Array,
    v: jax.Array,
):
    B, H, Sq, D = q.shape
    Sk = k.shape[2]
    BH = B * H
    hb = _heads_per_step(BH)
    steps = BH // hb

    q2 = q.reshape(BH, Sq, D)
    k2 = k.reshape(BH, Sk, D)
    v2 = v.reshape(BH, Sk, D)

    q_spec = pl.BlockSpec((hb, Sq, D), lambda i: (i, 0, 0))
    kv_spec = pl.BlockSpec((hb, Sk, D), lambda i: (i, 0, 0))

    out = pl.pallas_call(
        functools.partial(
            _attention_kernel, hb=hb, last=steps - 1, scale=float(D) ** -0.5
        ),
        grid=(steps,),
        in_specs=[q_spec, kv_spec, kv_spec],
        out_specs=pl.BlockSpec(memory_space=pl.ANY),
        out_shape=jax.ShapeDtypeStruct((BH, Sq, D), q.dtype),
        scratch_shapes=[
            pltpu.VMEM((BH, Sq, D), q.dtype),
            pltpu.SemaphoreType.DMA((2,)),
        ],
        compiler_params=pltpu.CompilerParams(
            dimension_semantics=("arbitrary",),
            vmem_limit_bytes=64 * 1024 * 1024,
        ),
    )(q2, k2, v2)
    return out.reshape(B, H, Sq, D)
```
